```python
import os as _os
_os.environ.setdefault('JAX_PLATFORMS', 'cpu')
import jax
import jax.numpy as jnp

def _softmax(x, axis=-1):
    return jax.nn.softmax(x, axis=axis)

def _gelu(x):
    return jax.nn.gelu(x, approximate=True)

def _silu(x):
    return jax.nn.silu(x)

def _sigmoid(x):
    return jax.nn.sigmoid(x)

def _layernorm(x, axis=-1, eps=1e-05):
    m = jnp.mean(x, axis=axis, keepdims=True)
    v = jnp.var(x, axis=axis, keepdims=True)
    return (x - m) / jnp.sqrt(v + eps)

def _scatter_add(tgt, idx, src, axis=0):
    return tgt.at[idx].add(src)

def _segment_sum(src, seg, n):
    return jax.ops.segment_sum(src, seg, n)

class _Rng:

    def __init__(self, key):
        self._k = key

    def _next(self):
        self._k, sub = jax.random.split(self._k)
        return sub

    def normal(self, shape):
        return jax.random.normal(self._next(), shape, dtype=jnp.bfloat16)

    def randint(self, lo, hi, shape):
        return jax.random.randint(self._next(), shape, lo, hi, dtype=jnp.int32)

    def uniform(self, shape, lo=0.0, hi=1.0):
        return jax.random.uniform(self._next(), shape, jnp.bfloat16, lo, hi)

    def permutation(self, n):
        return jax.random.permutation(self._next(), n)
kernel_name = 'adaLN_cond__linear_attn_block__swiglu_ffn__prompt'

def setup_inputs():
    _rng = _Rng(jax.random.key(int.from_bytes(__import__("os").urandom(4), "little")))
    _w = lambda a: (lambda t: t.astype(jnp.bfloat16) if jnp.issubdtype(t.dtype, jnp.floating) else t)(jnp.asarray(a))

    def _A_setup():
        B, S, D = (1, 2048, 640)
        return {'x': _w((lambda *s: _rng.normal(s) * 0.05)(B, S, D)), 'wqkv': _w((lambda *s: _rng.normal(s) * 0.8)(D, 3 * D)), 'wo': _w((lambda *s: _rng.normal(s) * 0.05)(D, D))}
    _A_in = _A_setup()

    def _B_setup():
        B, S, D, F = (1, 2048, 640, 1728)
        return {'x': _w((lambda *s: _rng.normal(s) * 0.05)(B, S, D)), 'w_gate': _w((lambda *s: _rng.normal(s) * 0.05)(D, F)), 'w_up': _w((lambda *s: _rng.normal(s) * 0.05)(D, F)), 'w_down': _w((lambda *s: _rng.normal(s) * 0.05)(F, D))}
    _B_in = _B_setup()
    return {'A_x': _A_in['x'], 'A_wqkv': _A_in['wqkv'], 'A_wo': _A_in['wo'], 'B_x': _B_in['x'], 'B_w_gate': _B_in['w_gate'], 'B_w_up': _B_in['w_up'], 'B_w_down': _B_in['w_down'], 'c': _w((lambda *s: _rng.normal(s) * 0.05)(1, 640) * 8.0), 'w_mod': _w((lambda *s: _rng.normal(s) * 0.05)(640, 6 * 640) * 640 ** (-0.5) * 8.0)}

def reference(A_x, A_wqkv, A_wo, B_x, B_w_gate, B_w_up, B_w_down, c, w_mod):

    def _A_ref(x, wqkv, wo):
        B, S, D = x.shape
        H = 32
        Dh = D // H
        qkv = (lambda x, *d: x.transpose(*d))((x @ wqkv).reshape(B, S, 3, H, Dh), 2, 0, 3, 1, 4)
        q, k, v = (qkv[0], qkv[1], qkv[2])
        phi = lambda t: jnp.where(t > 0, t + 1, jnp.exp(t)) + 1e-06
        pq, pk = (phi(q), phi(k))
        kv = jnp.einsum('bhsd,bhse->bhde', pk, v)
        z = jnp.einsum('bhsd->bhd', pk)
        num = jnp.einsum('bhqd,bhde->bhqe', pq, kv)
        den = jnp.einsum('bhqd,bhd->bhq', pq, z)[..., None] + 1e-06
        o = num / den
        return (lambda x, *d: x.transpose(*d))(o, 0, 2, 1, 3).reshape(B, S, D) @ wo

    def _B_ref(x, w_gate, w_up, w_down):
        g = _silu(x @ w_gate)
        u = x @ w_up
        return g * u @ w_down
    x = A_x
    mod = (_silu(c) @ w_mod).reshape(c.shape[0], 6, 1, -1)
    sa, ca, ga, sb, cb, gb = (mod[:, 0].copy(), mod[:, 1].copy(), mod[:, 2].copy(), mod[:, 3].copy(), mod[:, 4].copy(), mod[:, 5].copy())
    h = _layernorm(x, axis=-1) * (1 + ca) + sa
    x = x + ga * _A_ref(h, A_wqkv, A_wo)
    h = _layernorm(x, axis=-1) * (1 + cb) + sb
    x = x + gb * _B_ref(h, B_w_gate, B_w_up, B_w_down)
    return x
```

```python
import jax
import jax.numpy as jnp
from jax import lax
import jax.experimental.pallas as pl
import jax.experimental.pallas.tpu as pltpu

S, D, F, DH = 2048, 640, 1728, 20
T = 512
NB = S // T
FH, DQ = F // 2, D // 4
BF, F32, U32 = jnp.bfloat16, jnp.float32, jnp.uint32
SWAP = (0, 1, 0, 0, 1, 1, 1)
A2B = (0, 6, 1, 4, 5, 3, 2)
LONG = (0, 1, 2, 5)
WIDE = tuple(7 * p + q for p in LONG for q in LONG)
DEEP = tuple(7 * p + q for p in LONG for q in range(7))
PAIRS = ((0, 2), (1, 3), (4, None))
SPANS = ((0, 144), (112, 272), (240, 400), (368, 528), (496, 640))
RATE, LAG, XL = 2.1, 20, 20
GR, PR, RC = 80, 160, 192


def _dot(a, b):
    return jnp.dot(a, b, preferred_element_type=F32)


def _dot_nt(a, b):
    return lax.dot_general(a, b, (((1,), (1,)), ((), ())), preferred_element_type=F32)


def _add(a, b):
    return b if a is None else a if b is None else a + b


def _sub(a, b):
    return a if b is None else -b if a is None else a - b


_LHS7 = (lambda a, b, c, d: _add(a, d), lambda a, b, c, d: _add(c, d), lambda a, b, c, d: a, lambda a, b, c, d: d,
         lambda a, b, c, d: _add(a, b), lambda a, b, c, d: _sub(c, a), lambda a, b, c, d: _sub(b, d))
_RHS7 = (lambda a, b, c, d: _add(a, d), lambda a, b, c, d: a, lambda a, b, c, d: _sub(b, d), lambda a, b, c, d: _sub(c, a),
         lambda a, b, c, d: d, lambda a, b, c, d: _add(a, b), lambda a, b, c, d: _add(c, d))


def _out4(m1, m2, m3, m4, m5, m6, m7):
    return [[_add(_sub(_add(m1, m4), m5), m7), _add(m3, m5)], [_add(m2, m4), _add(_add(_sub(m1, m2), m3), m6)]]


def _one_level(forms, g):
    return {k: forms[k](*g[0], *g[1]) for k in range(7) if k in LONG or all(v is not None for row in g for v in row)}


def _two_levels(g, forms, ks, swap):
    outer, res = {}, {}
    for k in ks:
        p, q = divmod(k, 7)
        if p not in outer:
            outer[p] = [[forms[p](g[i][j], g[i][j + 2], g[i + 2][j], g[i + 2][j + 2]) for j in range(2)] for i in range(2)]
        o, s = outer[p], swap[p]
        res[k] = forms[q](o[0][s], o[0][1 - s], o[1][s], o[1][1 - s])
    return res


def _lhs49(g, ks=range(49)):
    return _two_levels(g, _LHS7, ks, (0,) * 7)


def _rhs49(g, ks=range(49)):
    return _two_levels(g, _RHS7, ks, SWAP)


def _out16(ms):
    inner = [_out4(*ms[7 * p:7 * p + 7]) for p in range(7)]
    out = [[None] * 4 for _ in range(4)]
    for i in range(2):
        for j in range(2):
            c = _out4(*[inner[p][i][j ^ SWAP[p]] for p in range(7)])
            for a in range(2):
                for b in range(2):
                    out[2 * a + i][2 * b + j] = c[a][b]
    return out


def _phi(t):
    return jnp.where(t > 0, t + 1.0, jnp.exp(t)) + 1e-6


def _tile(b):
    return slice(b * 128, (b + 1) * 128)


def _cat(xs, axis=0):
    return jnp.concatenate(xs, axis=axis)


def _pack(even, odd):
    return pltpu.pack_elementwise([even, odd], packed_dtype=BF)


def _half(x, e):
    return pltpu.unpack_elementwise(pltpu.bitcast(x, U32), index=e, packed_dtype=BF, unpacked_dtype=F32)


def _join(columns):
    return pltpu.bitcast(_cat([_cat(c) for c in columns], 1), BF)


def _zero(w):
    return (w == 1).astype(U32) & (w >> 1)


def _kernel(x_hbm, wqkv_hbm, wo_hbm, wgt_hbm, wut_hbm, wd_hbm, c_hbm, wmod_hbm, o_hbm,
            x_v, wqkv_v, wo_v, wgt_v, wut_v, wd_v, c_v, wmod_v, col_v, w2t_v, op_v, o_v, sem, osem):
    def cols(src, dst, lo, n, s):
        return pltpu.make_async_copy(src.at[:, pl.ds(lo, n)], dst.at[:, pl.ds(lo, n)], sem.at[s])

    def whole(src, dst, s):
        return pltpu.make_async_copy(src, dst, sem.at[s])

    loads = {'c': whole(c_hbm, c_v, 0), 'a': cols(wmod_hbm, wmod_v, 0, 2 * D, 1), 'b': cols(wmod_hbm, wmod_v, 2 * D, 4 * D, 2),
             'o': whole(wo_hbm, wo_v, 10), 'g': whole(wgt_hbm, wgt_v, 11), 'u': whole(wut_hbm, wut_v, 12), 'd': whole(wd_hbm, wd_v, 13)}
    loads.update({name: cols(wqkv_hbm, wqkv_v, j * D, D, 3 + j) for j, name in enumerate('qkv')})
    loads.update({str(i): whole(x_hbm.at[pl.ds(i * T, T)], x_v.at[pl.ds(i * T, T)], 6 + i) for i in range(NB)})

    def send(i, j):
        rows = pl.ds(i * T + j * T // 2, T // 2)
        return pltpu.make_async_copy(o_v.at[rows], o_hbm.at[rows], osem.at[2 * i + j])

    st = {}
    clock = {'mxu': 0.0, 'vpu': 0.0}
    pending, used = [], set()

    def book(ops, tie, key, values):
        clock['vpu'] = max(clock['vpu'], clock['mxu']) + ops / RATE
        if tie:
            pending.append((clock['vpu'] + LAG, key, values))

    def mark(values, ops, tie=False):
        book(ops + len(values), tie, None, [pltpu.bitcast(v, U32) for v in values[::4]] if tie else [])

    def put(name, r, columns, ops, tie=False, store=False):
        made = []
        for c, even, odd in columns:
            for k in even:
                st[name, k, r, c] = _pack(even[k], odd[k])
                made.append(st[name, k, r, c])
                if store:
                    where = ('kh'.index(name), 3 * k + c, slice(r // 2, r // 2 + 8), slice(None))
                    op_v[where] = made[-1]
                    st[name, k, r, c] = where
        if not store:
            book(ops + 2 * len(made), tie, (name, r, columns[0][0]), made)

    def words(name, k, r, n, c, m):
        used.update((name, rr, cc) for rr in range(r, r + n, 16) for cc in range(c, c + m))
        load = lambda w: op_v[w] if isinstance(w, tuple) else w
        return [[load(st[name, k, rr, cc]) for rr in range(r, r + n, 16)] for cc in range(c, c + m)]

    def matmul(lhs, rhs, dot=_dot):
        seen = None
        while pending and pending[0][0] <= clock['mxu']:
            _, key, made = pending.pop(0)
            if key not in used:
                for w in made:
                    seen = w if seen is None else seen | w
        if seen is not None:
            lhs = [[lhs[0][0] | _zero(seen)] + lhs[0][1:]] + lhs[1:]
        lhs = _join(lhs)
        out = dot(lhs, rhs)
        clock['mxu'] += (lhs.size * rhs.size * out.size) ** 0.5 / (4 * 128 * 128)
        return out

    def turn(tiles, tie=False):
        out = []
        for t in tiles:
            out.append(t.T)
            mark([out[-1][-32 // out[-1].dtype.itemsize:]], XL, tie)
        return _cat(out)

    def col(v):
        return jnp.broadcast_to(v, (128, D)).T

    def col_rows(j, r, e):
        return col_v[j, pl.ds(r + e, 8, stride=2), :]

    def mod_a():
        cf = c_v[...].astype(F32)
        st['sc'] = jnp.broadcast_to(cf * jax.nn.sigmoid(cf), (16, D)).astype(BF)
        mod = _dot(st['sc'], wmod_v[:, 0:2 * D])[0:1]
        col_v[0, 0:D] = col(mod[:, 0:D])
        col_v[1, 0:D] = col(1.0 + mod[:, D:2 * D])

    def mod_b():
        mod = _dot(st['sc'], wmod_v[:, 2 * D:6 * D])[0:1]
        st['ga'] = mod[:, 0:D]
        col_v[2, 0:D] = col(0.5 * mod[:, D:2 * D])
        col_v[3, 0:D] = col(0.5 * (1.0 + mod[:, 2 * D:3 * D]))
        col_v[5, 0:D] = col(2.0 * mod[:, 3 * D:4 * D])

    def proj_weights(name, tie=False, store=False):
        lo = 'qk'.index(name) * D
        wt = _cat([turn([wqkv_v[_tile(i), lo + j * 128:lo + (j + 1) * 128] for j in range(5)], tie) for i in range(5)], 1)
        cut = lambda v, t: None if t is None else v[:, _tile(t)]
        for r in range(0, DQ, 16):
            q = [[_half(wt[a * DQ + r:a * DQ + r + 16], e) for a in range(4)] for e in range(2)]
            for sub in range(2):
                put(name, sub * DQ + r, [(u, *[_one_level(_LHS7, [[cut(v, t) for t in pair] for v in h[sub::2]]) for h in q])
                                         for u, pair in enumerate(PAIRS)], 42, tie, store)

    def gate_up_weights(pieces=range(FH // 16), tie=False):
        for r in [(96 + 16 * j) % FH for j in pieces]:
            w = [ref[base + r:base + r + 16, :] for ref in (wgt_v, wut_v) for base in (0, FH)]
            q = [[_half(v, e) for v in w] for e in range(2)]
            main = [_lhs49([[v[:, _tile(j)] for j in range(4)] for v in h]) for h in q]
            more = [_lhs49([[v[:, 512:], None, None, None] for v in h], WIDE) for h in q]
            put('f', r, [(0, *main), (1, *more)], 220, tie)

    def down_weights(tie=False):
        for j in range(4):
            def piece(q):
                if j < 3:
                    base = (q // 2) * FH + 96 + 256 * j + 16 * (q % 2)
                    return turn([_cat([wd_v[base + 32 * m:base + 32 * m + 16, _tile(t)] for m in range(8)]) for t in range(5)], tie)
                return turn([_cat([wd_v[q * FH:q * FH + 96, _tile(t)], jnp.zeros((32, 128), BF)]) for t in range(5)], tie)
            wq = [piece(q) for q in range(4)] if j < 3 else [piece(0), piece(1), None, None]
            for r in range(0, DQ, 16):
                ops = [_lhs49([[None if w is None else _half(w[a * DQ + r:a * DQ + r + 16], e) * col_rows(5, a * DQ + r, e)
                                for w in wq] for a in range(4)], range(49) if j < 3 else DEEP) for e in range(2)]
                put('d', r, [(j, *ops)], 214 if j < 3 else 110, tie)

    def stats(x, tie):
        def total(f, ops):
            acc = None
            for r in range(0, D, 160):
                for j in range(r, r + 160, 8):
                    acc = _add(acc, f(x[j:j + 8]))
                mark([acc], 20 * ops, tie)
            return jnp.broadcast_to(jnp.sum(acc, axis=0, keepdims=True) * (1.0 / D), (8, 128))
        m = total(lambda v: v, 2)
        return m, lax.rsqrt(total(lambda v: (v - m) * (v - m), 3) + 1e-5)

    def normed(xs, stat, shift, scale):
        return lambda r, e, b: ((xs[b][e][r // 2:r // 2 + 8] - stat[b][0]) * stat[b][1] * col_rows(scale, r, e)
                                + col_rows(shift, r, e))

    def one_level_rhs(name, i, get, each, tie, store=False):
        at = lambda t, r, e, b: None if t is None else get(t * 128 + r, e, b)
        for u, pair in enumerate(PAIRS):
            for r in range(0, 128, 16):
                put(name, u * 128 + r, [(2 * i + j, *[_one_level(_RHS7, [[at(t, r, e, j), at(t, r, e, 2 + j)] for t in pair])
                                                      for e in range(2)]) for j in range(2)], 20 + 16 * each, tie, store)

    def load_x(i, tie=False):
        xt = [turn([x_v[i * T + b * 128:i * T + (b + 1) * 128, _tile(t)] for t in range(5)], tie) for b in range(4)]
        st['x', i] = [[_half(x, e) for e in range(2)] for x in xt]
        st['stat', i] = [stats(_cat(h), tie) for h in st['x', i]]

    def h_operands(i, tie=False, store=False):
        one_level_rhs('h', i, normed(st['x', i], st['stat', i], 0, 1), 3, tie, store)

    def project(name, i, steps=range(14)):
        for k, j in [divmod(n, 2) for n in steps]:
            u = 3 if k in LONG else 2
            st[(name, i), k, j] = _cat([matmul(words(name, k, r, PR, 0, u), _join(words('h', k, 0, 128 * u, 2 * i + j, 1)))
                                        for r in range(0, 2 * DQ, PR)])

    def result(key, r):
        c = [[_out4(*[st[key, k, j][sub * DQ + r:sub * DQ + r + 8] for k in range(7)]) for j in range(2)] for sub in range(2)]
        return [[c[a % 2][b % 2][a // 2][b // 2] for b in range(4)] for a in range(4)]

    def results(key, f, ops, tie):
        cs = []
        for r in range(0, DQ, 8):
            cs.append([[f(v) for v in row] for row in result(key, r)])
            mark([v for row in cs[-1] for v in row], ops, tie)
        return cs

    def k_operands(i, tie=False):
        for r in range(0, DQ, 16):
            pk = [[[_phi(v) for v in row] for row in result(('k', i), r + 8 * e)] for e in range(2)]
            for sub in range(2):
                ops = [[_one_level(_RHS7, [[p[sub][j], p[2 + sub][j]], [p[sub][2 + j], p[2 + sub][2 + j]]]) for p in pk]
                       for j in range(2)]
                put('p', sub * DQ + r, [(2 * i + j, *[{A2B[k]: v for k, v in o.items()} for o in ops[j]]) for j in range(2)], 164, tie)
            for e in range(2):
                for a, p in enumerate(pk[e]):
                    key = ('z', a * DQ + r + 8 * e)
                    st[key] = _add(st.get(key), (p[0] + p[1]) + (p[2] + p[3]))

    def z_total():
        z = _cat([st['z', r] for r in range(0, D, 8)])
        col_v[4, 0:D] = jnp.broadcast_to(jnp.sum(z, axis=1, keepdims=True), (D, 128))

    def gram(blocks):
        c, m = 2 * blocks[0], 2 * len(blocks)
        for k in range(7):
            for u in range(3 if k in LONG else 2):
                rhs = _join(words('h', k, 128 * u, 128, c, m))
                prod = _cat([matmul(words('p', k, r, GR, c, m), rhs, _dot_nt) for r in range(0, 2 * DQ, GR)])
                st['g', k, u] = _add(st.get(('g', k, u)), prod)
                clock['vpu'] += 40 * m / RATE

    def gram_result(tie=False):
        for r in range(0, 2 * DQ, 8):
            ms = [[st['g', A2B[p], u][r:r + 8] if ('g', A2B[p], u) in st else None for p in range(7)] for u in range(3)]
            c = [_out4(*ms[0]), _out4(*ms[1])]
            e = [_add(_sub(ms[2][0], ms[2][4]), ms[2][6]), _add(ms[2][2], ms[2][4])]
            for a in range(2):
                st['gr', 2 * a * DQ + r] = _cat([c[0][0][a], c[1][0][a], c[0][1][a], c[1][1][a], e[a]], 1)
            mark([v for q in c for row in q for v in row] + e, 19, tie)

    def kv():
        for j, (lo, hi) in enumerate(SPANS):
            clock['mxu'] += (hi - lo) * 5 / 4
            g = _cat([st['gr', r] for r in range(lo, hi, 8)]).astype(BF)
            full = _dot(g, wqkv_v[:, 2 * D + j * 128:2 * D + (j + 1) * 128])
            row = lax.broadcasted_iota(jnp.int32, full.shape, 0)
            row = lo + (row & -16) + ((row & 15) >> 1) + ((row & 1) << 3)
            head = (lax.broadcasted_iota(jnp.int32, full.shape, 1) + j * 128) // DH
            st['kv', j] = jnp.where(row // DH == head, full, 0.0).astype(BF)

    def out_weights(tie=False):
        for j, (lo, hi) in enumerate(SPANS):
            clock['mxu'] += (hi - lo) * 5 / 4
            part = _dot(st['kv', j], wo_v[_tile(j), :])
            for r in range(lo, hi, 16):
                st['w2', r] = _add(st.get(('w2', r)), part[r - lo:r - lo + 16])
        for j in range(5):
            w = _cat([st['w2', r] for r in range(j * 128, (j + 1) * 128, 16)]) * st['ga']
            w2t_v[j, 0:D] = turn([w[:, _tile(t)] for t in range(5)], tie)
        parts = {}
        for r in range(0, 2 * DQ, 8):
            w = [[w2t_v[j, pl.ds(2 * a * DQ + r // 16 * 16 + r % 16 // 8, 8, stride=2), :] for j in range(5)] for a in range(2)]
            for u, pair in enumerate(PAIRS):
                ops = _one_level(_LHS7, [[None if t is None else v[t] for t in pair] for v in w])
                for k, v in ops.items():
                    parts.setdefault((k, u), []).append(v)
                mark(list(ops.values()), 8, tie)
        st['w2t'] = [_cat([_cat(parts[k, u]) for u in range(3) if (k, u) in parts], 1).astype(BF) for k in range(7)]

    def q_operands(i, tie=False):
        sub = lax.broadcasted_iota(jnp.int32, (8, 128), 0)
        low = sub < 4
        cs = results(('q', i), _phi, 128, tie)
        out = []
        for pq in [_cat([c[a][b] for a in range(4) for c in cs]) for b in range(4)]:
            rows = []
            for r in range(0, D, 2 * DH):
                p = [pq[r + 8 * j:r + 8 * j + 8] for j in range(5)]
                t = [p[j] * col_v[4, r + 8 * j:r + 8 * j + 8, :] for j in range(5)]
                da = t[0] + t[1] + jnp.where(low, t[2], 0.0)
                db = t[3] + t[4] + jnp.where(low, 0.0, t[2])
                den = jnp.where(low, da + pltpu.roll(da, 4, 0), db + pltpu.roll(db, 4, 0))
                for step in (2, 1):
                    den = den + jnp.where((sub & step) == 0, pltpu.roll(den, 8 - step, 0), pltpu.roll(den, step, 0))
                den = den + 1e-6
                inv = pl.reciprocal(den, approx=True)
                inv = inv * (2.0 - den * inv)
                back = pltpu.roll(inv, 4, 0)
                ra, rb = jnp.where(low, inv, back), jnp.where(low, back, inv)
                rows += [p[j] * s for j, s in enumerate([ra, ra, inv, rb, rb])]
                mark(rows[-5:], 28, tie)
            out.append(rows)
        one_level_rhs('s', i, lambda r, e, b: out[b][r // 8 + e], 0, tie)

    def out_project(i, steps=range(14)):
        for k, j in [divmod(n, 2) for n in steps]:
            s = words('s', k, 0, 384 if k in LONG else 256, 2 * i + j, 1)
            st[('o', i), k, j] = matmul(s, st['w2t'][k], lambda rhs, w: _dot(w, rhs))

    def ffn_operands(i, tie=False):
        cs = results(('o', i), lambda v: v, 32, tie)
        x1 = [[st['x', i][b][e] + _cat([c[a][b] for a in range(4) for c in cs[e::2]]) for e in range(2)] for b in range(4)]
        st['x1', i] = [pltpu.bitcast(_pack(*h), BF) for h in x1]
        book(800, False, None, None)
        get = normed(x1, [stats(_cat(h), tie) for h in x1], 2, 3)
        for r in range(0, 128, 16):
            put('n', r, [(i, *[_rhs49([[get(j * 128 + r, e, b) for b in range(4)] for j in range(4)]) for e in range(2)])], 206, tie)
            put('n', 128 + r, [(i, *[_rhs49([[get(512 + r, e, b) for b in range(4)]] + [[None] * 4] * 3, WIDE)
                                     for e in range(2)])], 42, tie)

    chunks = [(r, RC) for r in range(96, FH, RC)] + [(0, 96)]

    def gate_up(i, steps=range(len(chunks))):
        for lo, rc in [chunks[n] for n in steps]:
            ms = [matmul(words('f', k, lo, rc, 0, 2 if k in WIDE else 1), _join(words('n', k, 0, 256 if k in WIDE else 128, i, 1)))
                  for k in range(49)]
            clock['vpu'] += rc * 24 / RATE

            def act(r):
                c = _out16([m[r:r + 8] for m in ms])
                return [[(c[a][b] + c[a][b] * jnp.tanh(c[a][b])) * c[a + 2][b] for b in range(4)] for a in range(2)]
            for r in range(0, rc, 8):
                if not lo:
                    ops = _rhs49(act(r) + [[None] * 4] * 2, DEEP)
                elif r % 32 < 16:
                    a0, a1 = act(r), act(r + 16)
                    ops = _rhs49([a0[0], a1[0], a0[1], a1[1]])
                else:
                    continue
                for k, v in ops.items():
                    st.setdefault(('act', i, k), []).append(v)

    def down(i, steps=range(49)):
        for k in steps:
            rhs = _cat(st.pop(('act', i, k)) + ([jnp.zeros((32, 128), F32)] if k in DEEP else [])).astype(BF)
            st['y', i, k] = matmul(words('d', k, 0, DQ, 0, rhs.shape[0] // 128), rhs)
            clock['vpu'] += 50 / RATE

    def finish(i, halves=(1, 0), tie=False):
        ys = [_out16([st['y', i, k][r:r + 8] if ('y', i, k) in st else None for k in range(49)]) for r in range(0, DQ, 8)]
        if tie:
            clock['vpu'] = clock['mxu']
            for c in ys:
                mark([c[a][b] for a in range(4) for j in halves for b in (2 * j, 2 * j + 1)], 20, tie)
        else:
            book(1300 * len(halves), False, None, None)
        for j in halves:
            for b in (2 * j, 2 * j + 1):
                y = st['x1', i][b] + _cat([c[a][b] for a in range(4) for c in ys])
                o_v[i * T + b * 128:i * T + (b + 1) * 128, :] = y.astype(BF).T
            send(i, j).start()

    def fetch(names):
        for name in names:
            loads[name].start()

    def wait(names):
        for name in names:
            loads[name].wait()

    fetch('0cak')
    fetch('q1')
    fetch('23')
    fetch('gu')
    fetch('bvod')
    wait('0')
    load_x(0)
    wait('ac')
    mod_a()
    h_operands(0, store=True)
    wait('k')
    proj_weights('k', store=True)
    clock['vpu'] = clock['mxu']
    project('k', 0, range(0, 12))
    wait('q1')
    proj_weights('q')
    load_x(1)
    project('k', 0, range(12, 14))
    k_operands(0)
    project('q', 0, range(0, 9))
    wait('23')
    project('q', 0, range(9, 14))
    h_operands(1, tie=True)
    project('k', 1)
    load_x(2)
    load_x(3, tie=True)
    h_operands(2)
    project('q', 1, range(0, 2))
    k_operands(1)
    h_operands(3)
    project('q', 1, range(2, 14))
    project('k', 2)
    k_operands(2)
    project('k', 3)
    k_operands(3, tie=True)
    wait('gu')
    project('q', 2, range(0, 10))
    z_total()
    gate_up_weights(tie=True)
    q_operands(0, tie=True)
    gram([0, 1])
    gram([2, 3])
    wait('bvod')
    mod_b()
    project('q', 2, range(10, 14))
    gram_result()
    kv()
    out_weights()
    out_project(0)
    project('q', 3, range(0, 6))
    ffn_operands(0)
    project('q', 3, range(6, 14))
    gate_up(0)
    down_weights(tie=True)
    q_operands(1)
    q_operands(2)
    out_project(1)
    down(0)
    ffn_operands(1)
    finish(0)
    gate_up(1)
    out_project(2)
    ffn_operands(2)
    down(1)
    finish(1)
    gate_up(2)
    q_operands(3)
    out_project(3)
    down(2)
    finish(2)
    ffn_operands(3)
    gate_up(3)
    down(3, range(0, 43))
    finish(3, (1,))
    down(3, range(43, 49))
    finish(3, (0,))
    for i in range(NB):
        for j in range(2):
            send(i, j).wait()


@jax.jit
def pallas_adaLN_cond__linear_attn_block__swiglu_ffn__prompt_kernel(
        A_x: jax.Array, A_wqkv: jax.Array, A_wo: jax.Array, B_x: jax.Array, B_w_gate: jax.Array,
        B_w_up: jax.Array, B_w_down: jax.Array, c: jax.Array, w_mod: jax.Array):
    hbm = pl.BlockSpec(memory_space=pl.ANY)
    vm = pltpu.VMEM
    out = pl.pallas_call(
        _kernel,
        out_shape=jax.ShapeDtypeStruct((S, D), BF),
        in_specs=[hbm] * 8,
        out_specs=hbm,
        scratch_shapes=[
            vm((S, D), BF), vm((D, 3 * D), BF), vm((D, D), BF), vm((F, D), BF), vm((F, D), BF), vm((F, D), BF),
            vm((1, D), BF), vm((D, 6 * D), BF),
            vm((6, D + 8, 128), F32), vm((5, D + 8, 128), F32), vm((2, 21, 192, 128), U32), vm((S, D), BF),
            pltpu.SemaphoreType.DMA((14,)), pltpu.SemaphoreType.DMA((2 * NB,)),
        ],
        compiler_params=pltpu.CompilerParams(vmem_limit_bytes=120 * 1024 * 1024),
    )(A_x.reshape(S, D), A_wqkv, A_wo, B_w_gate.T, B_w_up.T, B_w_down, c, w_mod)
    return out.reshape(1, S, D)
```
